```python
import jax
import jax.numpy as jnp

def _softmax(x, axis=-1):
    return jax.nn.softmax(x, axis=axis)
def _gelu(x):
    return jax.nn.gelu(x, approximate=True)
def _silu(x):
    return jax.nn.silu(x)
def _sigmoid(x):
    return jax.nn.sigmoid(x)
def _layernorm(x, axis=-1, eps=1e-5):
    m = jnp.mean(x, axis=axis, keepdims=True)
    v = jnp.var(x, axis=axis, keepdims=True)
    return (x - m) / jnp.sqrt(v + eps)
def _scatter_add(tgt, idx, src, axis=0):
    return tgt.at[idx].add(src)
def _segment_sum(src, seg, n):
    return jax.ops.segment_sum(src, seg, n)
class _Rng:
    def __init__(self, key):
        self._k = key
    def _next(self):
        self._k, sub = jax.random.split(self._k)
        return sub
    def normal(self, shape):
        return jax.random.normal(self._next(), shape, dtype=jnp.bfloat16)
    def randint(self, lo, hi, shape):
        return jax.random.randint(self._next(), shape, lo, hi, dtype=jnp.int32)
    def uniform(self, shape, lo=0.0, hi=1.0):
        return jax.random.uniform(self._next(), shape, jnp.bfloat16, lo, hi)
    def permutation(self, n):
        return jax.random.permutation(self._next(), n)


kernel_name = 'recurrent_scan__sliding_block_cached__dense_activation_gelu__decode'

def setup_inputs():
    _rng = _Rng(jax.random.key(int.from_bytes(__import__("os").urandom(4), "little")))
    _w = (lambda a: (lambda t: t.astype(jnp.bfloat16) if jnp.issubdtype(t.dtype, jnp.floating) else t)(jnp.asarray(a)))
    def _A_setup():
        B, Sq, D = 2, 1, 576
        Hq, Hkv, Sk, Dh = 32, 16, 32768, 128
        assert Hq % Hkv == 0, (Hq, Hkv)
        return {
            "x": _w((lambda *s: _rng.normal(s) * 0.05)(B, Sq, D)),
            "k_cache": _w((lambda *s: _rng.normal(s) * 0.05)(B, Hkv, Sk, Dh)),
            "v_cache": _w((lambda *s: _rng.normal(s) * 0.05)(B, Hkv, Sk, Dh)),
            "wq": _w((lambda *s: _rng.normal(s) * 0.05)(D, Hq * Dh) * (D ** -0.5)),
            "wo": _w((lambda *s: _rng.normal(s) * 0.05)(Hq * Dh, D) * ((Hq * Dh) ** -0.5)),
        }
    _A_in = _A_setup()

    def _B_setup():
        B, S, D, F = 2, 1, 576, 4608
        return {
            "x": _w((lambda *s: _rng.normal(s) * 0.05)(B, S, D)),
            "w1": _w((lambda *s: _rng.normal(s) * 0.05)(D, F) * (D ** -0.5)),
            "b1": _w((lambda *s: _rng.normal(s) * 0.05)(F) * 0.01),
            "w2": _w((lambda *s: _rng.normal(s) * 0.05)(F, D) * (F ** -0.5)),
            "b2": _w((lambda *s: _rng.normal(s) * 0.05)(D) * 0.01),
        }
    _B_in = _B_setup()

    return {
        "A_x": _A_in["x"],
        "A_k_cache": _A_in["k_cache"],
        "A_v_cache": _A_in["v_cache"],
        "A_wq": _A_in["wq"],
        "A_wo": _A_in["wo"],
        "B_x": _B_in["x"],
        "B_w1": _B_in["w1"],
        "B_b1": _B_in["b1"],
        "B_w2": _B_in["w2"],
        "B_b2": _B_in["b2"],
    }

def reference(A_x, A_k_cache, A_v_cache, A_wq, A_wo, B_x, B_w1, B_b1, B_w2, B_b2):
    def _A_ref(x, k_cache, v_cache, wq, wo):
        B, Sq, D = x.shape
        Hq, Dh = 32, 128
        Hkv, Sk = k_cache.shape[1], k_cache.shape[2]
        W = min(4096, max(256, Sk // 4))
        rep = Hq // Hkv
        q = (lambda x, *d: x.transpose(*d))((x @ wq).reshape(B, Sq, Hq, Dh), 0, 2, 1, 3)
        k = jnp.repeat(k_cache[:, :, Sk - W:, :], rep, axis=1)
        v = jnp.repeat(v_cache[:, :, Sk - W:, :], rep, axis=1)
        scores = jnp.einsum("bhqd,bhkd->bhqk", q, k) * (Dh ** -0.5)
        p = _softmax(scores, axis=-1)
        o = jnp.einsum("bhqk,bhkd->bhqd", p, v)
        return (lambda x, *d: x.transpose(*d))(o, 0, 2, 1, 3).reshape(B, Sq, Hq * Dh) @ wo

    def _B_ref(x, w1, b1, w2, b2):
        h = jnp.einsum("bsd,df->bsf", x, w1) + b1
        h = _gelu(h)
        return jnp.einsum("bsf,fd->bsd", h, w2) + b2

    x = A_x
    xn = _layernorm(x, axis=-1)
    s = _A_ref(xn, A_k_cache, A_v_cache, A_wq, A_wo)
    g = _silu(_B_ref(xn, B_w1, B_b1, B_w2, B_b2))
    return x + s * g
```

```python
import functools
import jax
import jax.numpy as jnp
from jax import lax
import jax.experimental.pallas as pl
import jax.experimental.pallas.tpu as pltpu

F32 = jnp.float32
BF16 = jnp.bfloat16
NT = (((1,), (1,)), ((), ()))


def _kernel(x_hbm, k_hbm, v_hbm, wq_hbm, wot_hbm, w1_hbm, b1_hbm, w2t_hbm, b2_hbm,
            out_ref,
            x_v, b1_v, b2_v, wq_v, w1_v, w2t_v, wot_v, kbuf, vbuf, q2, o2, b1f,
            sem_s, sem_w, sem_kv, *, W, CH, L, WCH):
    B, Hkv, Sk, Dh = k_hbm.shape
    D, F = w1_hbm.shape
    HD = wq_hbm.shape[1]
    Hq = HD // Dh
    NH = B * Hkv
    NS = L + 1

    def start_w(src, dst, sem):
        n = D // WCH
        for c in range(n):
            pltpu.make_async_copy(src.at[pl.ds(c * WCH, WCH)], dst.at[pl.ds(c * WCH, WCH)], sem).start(priority=c % 2)

    def wait_all(dst, sem):
        pltpu.make_async_copy(dst, dst, sem).wait()

    def start_kv(i, slot):
        b = lax.shift_right_logical(i, 4)
        h = i & (Hkv - 1)
        for c in range(W // CH):
            src = pl.ds(Sk - W + c * CH, CH)
            dst = pl.ds(c * CH, CH)
            pltpu.make_async_copy(k_hbm.at[b, h, src], kbuf.at[slot, dst], sem_kv.at[0, slot]).start(priority=0)
            pltpu.make_async_copy(v_hbm.at[b, h, src], vbuf.at[slot, dst], sem_kv.at[1, slot]).start(priority=1)

    cx = pltpu.make_async_copy(x_hbm, x_v, sem_s.at[0]); cx.start()
    start_w(wq_hbm, wq_v, sem_w.at[0])
    cb1 = pltpu.make_async_copy(b1_hbm, b1_v, sem_s.at[1]); cb1.start()
    cb2 = pltpu.make_async_copy(b2_hbm, b2_v, sem_s.at[2]); cb2.start()
    start_w(w1_hbm, w1_v, sem_w.at[1])

    cx.wait()
    x = x_v[...].astype(F32)
    m = jnp.mean(x, axis=-1, keepdims=True)
    xc = x - m
    var = jnp.mean(xc * xc, axis=-1, keepdims=True)
    xn = xc / jnp.sqrt(var + 1e-5)
    xn8 = jnp.concatenate([xn, jnp.zeros((8 - B, D), F32)], axis=0).astype(BF16)

    wait_all(wq_v, sem_w.at[0])
    start_w(w2t_hbm, w2t_v, sem_w.at[2])
    q = jnp.dot(xn8, wq_v[...], preferred_element_type=F32)
    for j in range(Hq):
        q2[pl.ds(j, B, stride=Hq), :] = q[0:B, j * Dh:(j + 1) * Dh]

    wait_all(w1_v, sem_w.at[1])
    for i in range(L):
        start_kv(jnp.int32(i), i)
    cb1.wait()
    b1f[...] = b1_v[...].astype(F32)
    h1 = jnp.dot(xn8, w1_v[...], preferred_element_type=F32)
    bias1 = jnp.concatenate([jnp.broadcast_to(b1f[pl.ds(j, 1), :], (8, 128)) for j in range(F // 128)], axis=1)
    hg = jax.nn.gelu(h1 + bias1, approximate=True).astype(BF16)

    wait_all(w2t_v, sem_w.at[2])
    cb2.wait()
    y = lax.dot_general(hg, w2t_v[...], NT, preferred_element_type=F32)
    y = y[0:B] + b2_v[...].astype(F32).reshape(1, D)
    g = y * jax.nn.sigmoid(y)

    o2[...] = jnp.zeros(o2.shape, F32)
    scale = Dh ** -0.5
    row = lax.broadcasted_iota(jnp.int32, (8, Dh), 0)

    def body(i, carry):
        slot = lax.rem(i, NS)
        nxt = i + L
        @pl.when(nxt < NH)
        def _():
            start_kv(nxt, lax.rem(nxt, NS))
        @pl.when(nxt == NH)
        def _():
            start_w(wot_hbm, wot_v, sem_w.at[3])
        grp = pl.multiple_of(lax.shift_right_logical(i, 2) * 8, 8)
        qg = q2[pl.ds(grp, 8), :].astype(BF16)
        wait_all(kbuf.at[slot], sem_kv.at[0, slot])
        s = lax.dot_general(qg, kbuf[slot], NT, preferred_element_type=F32) * scale
        mx = jnp.max(s, axis=-1, keepdims=True)
        p = jnp.exp(s - mx)
        l = jnp.sum(p, axis=-1, keepdims=True)
        wait_all(vbuf.at[slot], sem_kv.at[1, slot])
        o = jnp.dot(p.astype(BF16), vbuf[slot], preferred_element_type=F32) / l
        sel = lax.shift_right_logical(row, 1) == (i & 3)
        o2[pl.ds(grp, 8), :] = jnp.where(sel, o, o2[pl.ds(grp, 8), :])
        return carry

    lax.fori_loop(0, NH, body, 0)

    zpad = jnp.zeros((8 - B, Dh), F32)
    oc = jnp.concatenate(
        [jnp.concatenate([o2[pl.ds(j, B, stride=Hq), :], zpad], axis=0) for j in range(Hq)], axis=1).astype(BF16)
    wait_all(wot_v, sem_w.at[3])
    sres = lax.dot_general(oc, wot_v[...], NT, preferred_element_type=F32)[0:B]
    out_ref[...] = (x + sres * g).astype(out_ref.dtype)


@jax.jit
def pallas_recurrent_scan__sliding_block_cached__dense_activation_gelu__decode_kernel(A_x, A_k_cache, A_v_cache, A_wq, A_wo, B_x, B_w1, B_b1, B_w2, B_b2):
    CH, L, WCH = 128, 2, 16
    B, Sq, D = A_x.shape
    _, Hkv, Sk, Dh = A_k_cache.shape
    W = min(4096, max(256, Sk // 4))
    HD = A_wq.shape[1]
    F = B_w1.shape[1]
    any_spec = pl.BlockSpec(memory_space=pl.ANY)
    out = pl.pallas_call(
        functools.partial(_kernel, W=W, CH=CH, L=L, WCH=WCH),
        in_specs=[any_spec] * 9,
        out_specs=pl.BlockSpec(memory_space=pltpu.VMEM),
        out_shape=jax.ShapeDtypeStruct((B, D), A_x.dtype),
        scratch_shapes=[
            pltpu.VMEM((B, D), BF16),
            pltpu.VMEM((F // 128, 128), BF16),
            pltpu.VMEM((D,), BF16),
            pltpu.VMEM((D, HD), BF16),
            pltpu.VMEM((D, F), BF16),
            pltpu.VMEM((D, F), BF16),
            pltpu.VMEM((D, HD), BF16),
            pltpu.VMEM((L + 1, W, Dh), BF16),
            pltpu.VMEM((L + 1, W, Dh), BF16),
            pltpu.VMEM((B * HD // Dh, Dh), F32),
            pltpu.VMEM((B * HD // Dh, Dh), F32),
            pltpu.VMEM((F // 128, 128), F32),
            pltpu.SemaphoreType.DMA((3,)),
            pltpu.SemaphoreType.DMA((4,)),
            pltpu.SemaphoreType.DMA((2, L + 1)),
        ],
        compiler_params=pltpu.CompilerParams(vmem_limit_bytes=64 * 2**20, disable_bounds_checks=True),
    )(A_x.reshape(B, D), A_k_cache, A_v_cache, A_wq, A_wo.T, B_w1, B_b1.reshape(F // 128, 128), B_w2.T, B_b2)
    return out.reshape(B, Sq, D)
```

```python
import functools
import jax
import jax.numpy as jnp
from jax import lax
import jax.experimental.pallas as pl
import jax.experimental.pallas.tpu as pltpu

F32 = jnp.float32
BF16 = jnp.bfloat16
NT = (((1,), (1,)), ((), ()))
NP = 4
CB = 512
RB = 8
CPG = 8


def _kernel(x_hbm, k_hbm, v_hbm, wq_hbm, wot_hbm, w1_hbm, b1_hbm, w2t_hbm, b2_hbm,
            out_ref,
            x_v, b1_v, b2_v, wq_v, w1_v, w2t_v, wot_v, kbuf, vbuf,
            xn_s, q2, o2, b1f, h_s, y_s, s_s, p_s, l_s,
            sem, *, W, KR, LOOK, EX, TAIL, NOCOMP, UW, UK, SH):
    NG, _, Sk, Dh = k_hbm.shape
    _, R, F = w1_hbm.shape
    HD = wq_hbm.shape[2]
    B, D = x_v.shape
    NSEM = sem.shape[0]
    Hq = HD // Dh
    NB = R // RB
    CR = W // CPG
    nq, nf = HD // CB, F // CB
    TB0 = NB // 2
    TC0 = TB0 + NG * CPG
    TE0 = TC0 + nq
    assert sum(TAIL) == F - HD and LOOK + EX <= NSEM
    nc = 'qhasy' if NOCOMP is True else (NOCOMP or '')

    def loop(lo, hi, fn, unroll=1):
        lax.fori_loop(lo, hi, lambda i, c: (fn(i), c)[1], 0, unroll=unroll)

    def wcopy(src, dst, band, c0, cw, q, slot):
        sl = (slice(None), pl.ds(pl.multiple_of(band * RB, RB), RB), pl.ds(c0, cw))
        pltpu.make_async_copy(src.at[sl], dst.at[sl], sem.at[slot]).start(priority=q)

    def ycol(e):
        return pl.multiple_of(((e + SH) & (nq - 1)) * CB, CB)

    def issue(t):
        slot = t & (NSEM - 1)

        @pl.when(t < TB0)
        def _():
            def f(i):
                for j in range(nf):
                    if j < nq:
                        wcopy(wq_hbm, wq_v, t * 2 + i, j * CB, CB, 0, slot)
                    wcopy(w1_hbm, w1_v, t * 2 + i, j * CB, CB, 1, slot)
            loop(0, 2, f)

        @pl.when((t >= TB0) & (t < TC0))
        def _():
            u = t - TB0
            g = lax.shift_right_logical(u, 3)
            base = (u & (CPG - 1)) * CR
            def f(i):
                off = pl.multiple_of(base + i * KR, KR)
                src = pl.ds(Sk - W + off, KR)
                dst = pl.ds(off, KR)
                pltpu.make_async_copy(k_hbm.at[g, :, src], kbuf.at[g & 3, :, dst], sem.at[slot]).start(priority=0)
                pltpu.make_async_copy(v_hbm.at[g, :, src], vbuf.at[g & 3, :, dst], sem.at[slot]).start(priority=1)
            loop(0, CR // KR, f, UK)

        @pl.when((t >= TC0) & (t < TE0))
        def _():
            def f(i):
                wcopy(wot_hbm, wot_v, i, pl.multiple_of((t - TC0) * CB, CB), CB, 0, slot)
                wcopy(w2t_hbm, w2t_v, i, ycol(t - TC0), CB, 1, slot)
            loop(0, NB, f, UW)

        c0 = HD
        for i, cw in enumerate(TAIL):
            @pl.when(t == TE0 + i)
            def _():
                def f(i):
                    wcopy(w2t_hbm, w2t_v, i, c0, cw, 0, slot)
                    wcopy(w2t_hbm, w2t_v, i + NB // 2, c0, cw, 1, slot)
                loop(0, NB // 2, f, UW)
            c0 += cw

    def wait_on(d, slot):
        pltpu.make_async_copy(d, d, sem.at[slot]).wait()

    def wait(t):
        slot = t & (NSEM - 1)

        @pl.when(t < TB0)
        def _():
            rows = pl.ds(pl.multiple_of(t * 2 * RB, 2 * RB), 2 * RB)
            wait_on(wq_v.at[:, rows], slot)
            wait_on(w1_v.at[:, rows], slot)

        @pl.when((t >= TB0) & (t < TC0))
        def _():
            u = t - TB0
            g = lax.shift_right_logical(u, 3)
            rows = pl.ds(pl.multiple_of((u & (CPG - 1)) * CR, CR), CR)
            wait_on(kbuf.at[g & 3, :, rows], slot)
            wait_on(vbuf.at[g & 3, :, rows], slot)

        @pl.when(t >= TC0)
        def _():
            wait_on(wot_v.at[:, :, pl.ds(pl.multiple_of((t - TC0) * CB, CB), CB)], slot)
            wait_on(w2t_v.at[:, :, pl.ds(ycol(t - TC0), CB)], slot)

    small = [pltpu.make_async_copy(s, d, sem.at[LOOK - 1])
             for s, d in ((x_hbm, x_v), (b1_hbm, b1_v), (b2_hbm, b2_v))]
    loop(0, LOOK, issue)
    for c in small:
        c.start()
    s_s[...] = jnp.zeros(s_s.shape, F32)
    o2[...] = jnp.zeros(o2.shape, F32)
    scale = Dh ** -0.5
    TPB = CB // Dh

    def prologue():
        for c in small:
            c.wait()
        x = x_v[...].astype(F32)
        m = jnp.mean(x, axis=-1, keepdims=True)
        xc = x - m
        var = jnp.mean(xc * xc, axis=-1, keepdims=True)
        xn = xc / jnp.sqrt(var + 1e-5)
        xn_s[...] = jnp.concatenate([xn, jnp.zeros((16 - B, D), F32)], axis=0).astype(BF16)
        b1f[...] = b1_v[...].astype(F32)
        y_s[...] = jnp.broadcast_to(b2_v[...].astype(F32).reshape(1, D), (8, D))

    def q_piece(j):
        w = wq_v[:, :, pl.ds(pl.multiple_of(j * CB, CB), CB)].reshape(D, CB)
        q = jnp.dot(xn_s[...], w, preferred_element_type=F32)
        for i in range(TPB):
            q2[pl.ds(j * TPB + i, B, stride=Hq), :] = q[0:B, i * Dh:(i + 1) * Dh]

    def h_piece(j):
        cols = pl.ds(pl.multiple_of(j * CB, CB), CB)
        w = w1_v[:, :, cols].reshape(D, CB)
        h = jnp.dot(xn_s[...], w, preferred_element_type=F32)
        bias = jnp.concatenate(
            [jnp.broadcast_to(b1f[pl.ds(j * TPB + i, 1), :], (16, Dh)) for i in range(TPB)], axis=1)
        h_s[:, cols] = jax.nn.gelu(h + bias, approximate=True).astype(BF16)

    def y_part(c0, cw):
        w = w2t_v[:, :, pl.ds(c0, cw)].reshape(D, cw)
        return lax.dot_general(h_s[:, pl.ds(c0, cw)], w, NT, preferred_element_type=F32)[0:8]

    def s_part(j):
        w = wot_v[:, :, pl.ds(pl.multiple_of(j * CB, CB), CB)].reshape(D, CB)
        zpad = jnp.zeros((8 - B, Dh), F32)
        oc = jnp.concatenate(
            [jnp.concatenate([o2[pl.ds(j * TPB + i, B, stride=Hq), :], zpad], axis=0) for i in range(TPB)],
            axis=1).astype(BF16)
        return lax.dot_general(oc, w, NT, preferred_element_type=F32)

    def half(u):
        hd = lax.shift_right_logical(u, 1)
        g = lax.shift_right_logical(hd, 2)
        j = hd & 3
        rows = pl.ds(pl.multiple_of(g * 8, 8), 8)

        @pl.when((u & 1) == 0)
        def _():
            qg = q2[rows, :].astype(BF16)
            s = lax.dot_general(qg, kbuf[g & 3, j], NT, preferred_element_type=F32) * scale
            mx = jnp.max(s, axis=-1, keepdims=True)
            p = jnp.exp(s - mx)
            l_s[...] = jnp.broadcast_to(jnp.sum(p, axis=-1, keepdims=True), l_s.shape)
            p_s[...] = p

        @pl.when((u & 1) == 1)
        def _():
            o = jnp.dot(p_s[...].astype(BF16), vbuf[g & 3, j], preferred_element_type=F32) / l_s[...]
            row = lax.broadcasted_iota(jnp.int32, (8, Dh), 0)
            o2[rows, :] = jnp.where(lax.shift_right_logical(row, 1) == j, o, o2[rows, :])

    def tgt(t):
        return t + 1 + LOOK + jnp.clip(t + LOOK - TC0, 0, EX)

    def step(t):
        with jax.named_scope("wait"):
            wait(t)
        with jax.named_scope("issue"):
            if EX:
                loop(tgt(t - 1), tgt(t), issue)
            else:
                issue(t + LOOK)
        b = t - TB0

        @pl.when(t == LOOK - 1)
        def _():
            prologue()

        @pl.when((b >= 0) & (b < nq))
        def _():
            if 'q' not in nc: q_piece(b)

        @pl.when((b >= 0) & (b < nf))
        def _():
            if 'h' not in nc: h_piece(b)

        nh = NG * CPG
        lo = jnp.where(b < nh, b - CPG, 2 * b - nh - CPG + 2)
        hi = jnp.where(b < nh - 1, b - CPG + 1, 2 * b - nh - CPG + 4)
        if 'a' not in nc: loop(jnp.clip(lo, 0, nh), jnp.clip(hi, 0, nh), half)

        @pl.when(t >= TC0)
        def _():
            if 's' not in nc: s_s[...] += s_part(t - TC0)
            if 'y' not in nc: y_s[...] += y_part(ycol(t - TC0), CB)

    loop(0, TE0, step)

    y = y_s[...]
    c0 = HD
    for i, cw in enumerate(TAIL):
        wait_on(w2t_v.at[:, :, pl.ds(c0, cw)], (TE0 + i) & (NSEM - 1))
        if 'y' not in nc: y = y + y_part(c0, cw)
        c0 += cw
    y = y[0:B]
    g = y * jax.nn.sigmoid(y)
    out_ref[...] = (x_v[...].astype(F32) + s_s[0:B, :] * g).astype(out_ref.dtype)


@jax.jit
def pallas_recurrent_scan__sliding_block_cached__dense_activation_gelu__decode_kernel(A_x, A_k_cache, A_v_cache, A_wq, A_wo, B_x, B_w1, B_b1, B_w2, B_b2):
    KR = 32
    LOOK = 3
    EX = 0
    TAIL = (512,)
    NOCOMP = False
    UW = 3
    UK = 1
    NSEM = 4
    SH = 0
    B, Sq, D = A_x.shape
    _, Hkv, Sk, Dh = A_k_cache.shape
    W = min(4096, max(256, Sk // 4))
    HD = A_wq.shape[1]
    F = B_w1.shape[1]
    R = D // NP
    NG = B * Hkv // NP
    any_spec = pl.BlockSpec(memory_space=pl.ANY)
    out = pl.pallas_call(
        functools.partial(_kernel, W=W, KR=KR, LOOK=LOOK, EX=EX, TAIL=TAIL, NOCOMP=NOCOMP, UW=UW, UK=UK, SH=SH),
        in_specs=[any_spec] * 9,
        out_specs=pl.BlockSpec(memory_space=pltpu.VMEM),
        out_shape=jax.ShapeDtypeStruct((B, D), A_x.dtype),
        scratch_shapes=[
            pltpu.VMEM((B, D), BF16),
            pltpu.VMEM((F // 128, 128), BF16),
            pltpu.VMEM((D,), BF16),
            pltpu.VMEM((NP, R, HD), BF16),
            pltpu.VMEM((NP, R, F), BF16),
            pltpu.VMEM((NP, R, F), BF16),
            pltpu.VMEM((NP, R, HD), BF16),
            pltpu.VMEM((4, NP, W, Dh), BF16),
            pltpu.VMEM((4, NP, W, Dh), BF16),
            pltpu.VMEM((16, D), BF16),
            pltpu.VMEM((B * HD // Dh, Dh), F32),
            pltpu.VMEM((B * HD // Dh, Dh), F32),
            pltpu.VMEM((F // 128, 128), F32),
            pltpu.VMEM((16, F), BF16),
            pltpu.VMEM((8, D), F32),
            pltpu.VMEM((8, D), F32),
            pltpu.VMEM((8, W), F32),
            pltpu.VMEM((8, Dh), F32),
            pltpu.SemaphoreType.DMA((NSEM,)),
        ],
        compiler_params=pltpu.CompilerParams(vmem_limit_bytes=80 * 2**20, disable_bounds_checks=True),
    )(A_x.reshape(B, D), A_k_cache.reshape(NG, NP, Sk, Dh), A_v_cache.reshape(NG, NP, Sk, Dh),
      A_wq.reshape(NP, R, HD), A_wo.T.reshape(NP, R, HD), B_w1.reshape(NP, R, F),
      B_b1.reshape(F // 128, 128), B_w2.T.reshape(NP, R, F), B_b2)
    return out.reshape(B, Sq, D)
```

```python
import functools
import jax
import jax.numpy as jnp
from jax import lax
import jax.experimental.pallas as pl
import jax.experimental.pallas.tpu as pltpu

F32 = jnp.float32
BF16 = jnp.bfloat16
NT = (((1,), (1,)), ((), ()))
NP = 4
CB = 512
RB = 8
CPG = 8


def _kernel(x_hbm, k_hbm, v_hbm, wq_hbm, wot_hbm, w1_hbm, b1_hbm, w2t_hbm, b2_hbm,
            out_ref,
            x_v, b1_v, b2_v, wq_v, w1_v, w2t_v, wot_v, kbuf, vbuf,
            xn_s, q2, o2, b1f, h_s, y_s, s_s, p_s, l_s,
            sem, *, W, KR, LOOK, EX, TAIL, NOCOMP, UW, UK, SH, ORD):
    NG, _, Sk, Dh = k_hbm.shape
    _, R, F = w1_hbm.shape
    HD = wq_hbm.shape[2]
    B, D = x_v.shape
    NSEM = 4
    Hq = HD // Dh
    NB = R // RB
    CR = W // CPG
    nq, nf = HD // CB, F // CB
    TB0 = NB // 2
    TC0 = TB0 + NG * CPG
    TD0 = TC0 + nq // 2
    TE0 = TC0 + nq
    assert sum(TAIL) == F - HD and LOOK + EX <= NSEM
    nc = 'qhasy' if NOCOMP is True else (NOCOMP or '')

    def loop(lo, hi, fn, unroll=1):
        lax.fori_loop(lo, hi, lambda i, c: (fn(i), c)[1], 0, unroll=unroll)

    def wcopy(src, dst, band, c0, cw, q, slot):
        sl = (slice(None), pl.ds(pl.multiple_of(band * RB, RB), RB), pl.ds(c0, cw))
        pltpu.make_async_copy(src.at[sl], dst.at[sl], sem.at[slot]).start(priority=q)

    def ycol(e):
        return pl.multiple_of(((e + SH) & (nq - 1)) * CB, CB)

    last = [(HD - 2 * CB, CB, (TE0 - 1) & 3), (HD - CB, CB, TE0 & 3),
            (HD, TAIL[0], (TE0 + 1) & 3), (HD + TAIL[0], TAIL[1], 4)]

    def issue(t):
        slot = t & (NSEM - 1)

        @pl.when(t < TB0)
        def _():
            def f(i):
                for j in range(nf):
                    if j < nq:
                        wcopy(wq_hbm, wq_v, t * 2 + i, j * CB, CB, 0, slot)
                    wcopy(w1_hbm, w1_v, t * 2 + i, j * CB, CB, 1, slot)
            loop(0, 2, f)

        @pl.when((t >= TB0) & (t < TC0))
        def _():
            u = t - TB0
            g = lax.shift_right_logical(u, 3)
            base = (u & (CPG - 1)) * CR
            def f(i):
                off = pl.multiple_of(base + i * KR, KR)
                src = pl.ds(Sk - W + off, KR)
                dst = pl.ds(off, KR)
                pltpu.make_async_copy(k_hbm.at[g, :, src], kbuf.at[g & 3, :, dst], sem.at[slot]).start(priority=0)
                pltpu.make_async_copy(v_hbm.at[g, :, src], vbuf.at[g & 3, :, dst], sem.at[slot]).start(priority=1)
            loop(0, CR // KR, f, UK)

        for src, dst, t0 in ((wot_hbm, wot_v, TC0), (w2t_hbm, w2t_v, TD0)):
            @pl.when((t >= t0) & (t < min(t0 + nq // 2, TE0 - 1)))
            def _():
                def f(i):
                    for q in range(2):
                        wcopy(src, dst, i, pl.multiple_of(((t - t0) * 2 + q) * CB, CB), CB, q, slot)
                loop(0, NB, f, UW)

        for i in range(0, len(last), 2):
            @pl.when(t == TE0 - 1 + i // 2)
            def _():
                def f(r):
                    for q in range(2):
                        c0, cw, sl = last[i + q]
                        wcopy(w2t_hbm, w2t_v, r, c0, cw, q, sl)
                loop(0, NB, f, UW)

    def wait_on(d, slot):
        pltpu.make_async_copy(d, d, sem.at[slot]).wait()

    def wait(t):
        slot = t & (NSEM - 1)

        @pl.when(t < TB0)
        def _():
            rows = pl.ds(pl.multiple_of(t * 2 * RB, 2 * RB), 2 * RB)
            wait_on(wq_v.at[:, rows], slot)
            wait_on(w1_v.at[:, rows], slot)

        @pl.when((t >= TB0) & (t < TC0))
        def _():
            u = t - TB0
            g = lax.shift_right_logical(u, 3)
            rows = pl.ds(pl.multiple_of((u & (CPG - 1)) * CR, CR), CR)
            wait_on(kbuf.at[g & 3, :, rows], slot)
            wait_on(vbuf.at[g & 3, :, rows], slot)

        for dst, t0 in ((wot_v, TC0), (w2t_v, TD0)):
            @pl.when((t >= t0) & (t < t0 + nq // 2))
            def _():
                wait_on(dst.at[:, :, pl.ds(pl.multiple_of((t - t0) * 2 * CB, 2 * CB), 2 * CB)], slot)

    small = [pltpu.make_async_copy(s, d, sem.at[LOOK - 1])
             for s, d in ((x_hbm, x_v), (b1_hbm, b1_v), (b2_hbm, b2_v))]
    loop(0, LOOK, issue)
    for c in small:
        c.start()
    s_s[...] = jnp.zeros(s_s.shape, F32)
    o2[...] = jnp.zeros(o2.shape, F32)
    scale = Dh ** -0.5
    TPB = CB // Dh

    def prologue():
        for c in small:
            c.wait()
        x = x_v[...].astype(F32)
        m = jnp.mean(x, axis=-1, keepdims=True)
        xc = x - m
        var = jnp.mean(xc * xc, axis=-1, keepdims=True)
        xn = xc / jnp.sqrt(var + 1e-5)
        xn_s[...] = jnp.concatenate([xn, jnp.zeros((16 - B, D), F32)], axis=0).astype(BF16)
        b1f[...] = b1_v[...].astype(F32)
        y_s[...] = jnp.broadcast_to(b2_v[...].astype(F32).reshape(1, D), (8, D))

    def q_piece(j):
        w = wq_v[:, :, pl.ds(pl.multiple_of(j * CB, CB), CB)].reshape(D, CB)
        q = jnp.dot(xn_s[...], w, preferred_element_type=F32)
        for i in range(TPB):
            q2[pl.ds(j * TPB + i, B, stride=Hq), :] = q[0:B, i * Dh:(i + 1) * Dh]

    def h_piece(j):
        cols = pl.ds(pl.multiple_of(j * CB, CB), CB)
        w = w1_v[:, :, cols].reshape(D, CB)
        h = jnp.dot(xn_s[...], w, preferred_element_type=F32)
        bias = jnp.concatenate(
            [jnp.broadcast_to(b1f[pl.ds(j * TPB + i, 1), :], (16, Dh)) for i in range(TPB)], axis=1)
        h_s[:, cols] = jax.nn.gelu(h + bias, approximate=True).astype(BF16)

    def y_part(c0, cw):
        w = w2t_v[:, :, pl.ds(c0, cw)].reshape(D, cw)
        return lax.dot_general(h_s[:, pl.ds(c0, cw)], w, NT, preferred_element_type=F32)[0:8]

    def s_part(j):
        w = wot_v[:, :, pl.ds(pl.multiple_of(j * 2 * CB, 2 * CB), 2 * CB)].reshape(D, 2 * CB)
        zpad = jnp.zeros((8 - B, Dh), F32)
        oc = jnp.concatenate(
            [jnp.concatenate([o2[pl.ds(j * 2 * TPB + i, B, stride=Hq), :], zpad], axis=0) for i in range(2 * TPB)],
            axis=1).astype(BF16)
        return lax.dot_general(oc, w, NT, preferred_element_type=F32)

    def half(u):
        hd = lax.shift_right_logical(u, 1)
        g = lax.shift_right_logical(hd, 2)
        j = hd & 3
        rows = pl.ds(pl.multiple_of(g * 8, 8), 8)

        @pl.when((u & 1) == 0)
        def _():
            qg = q2[rows, :].astype(BF16)
            s = lax.dot_general(qg, kbuf[g & 3, j], NT, preferred_element_type=F32) * scale
            mx = jnp.max(s, axis=-1, keepdims=True)
            p = jnp.exp(s - mx)
            l_s[...] = jnp.broadcast_to(jnp.sum(p, axis=-1, keepdims=True), l_s.shape)
            p_s[...] = p

        @pl.when((u & 1) == 1)
        def _():
            o = jnp.dot(p_s[...].astype(BF16), vbuf[g & 3, j], preferred_element_type=F32) / l_s[...]
            row = lax.broadcasted_iota(jnp.int32, (8, Dh), 0)
            o2[rows, :] = jnp.where(lax.shift_right_logical(row, 1) == j, o, o2[rows, :])

    def tgt(t):
        return t + 1 + LOOK + jnp.clip(t + LOOK - TC0, 0, EX)

    def step(t):
        if True:
            wait(t)
        if True:
            if EX:
                loop(tgt(t - 1), tgt(t), issue)
            else:
                issue(t + LOOK)
        b = t - TB0

        @pl.when(t == LOOK - 1)
        def _():
            prologue()

        @pl.when((b >= 0) & (b < nq))
        def _():
            if 'q' not in nc: q_piece(b)

        @pl.when((b >= 0) & (b < nf))
        def _():
            if 'h' not in nc: h_piece(b)

        nh = NG * CPG
        lo = jnp.where(b < nh, b - CPG, 2 * b - nh - CPG + 2)
        hi = jnp.where(b < nh - 1, b - CPG + 1, 2 * b - nh - CPG + 4)
        if 'a' not in nc: loop(jnp.clip(lo, 0, nh), jnp.clip(hi, 0, nh), half)

        @pl.when((t >= TC0) & (t < TD0))
        def _():
            if 's' not in nc: s_s[...] += s_part(t - TC0)

        @pl.when(t >= TD0)
        def _():
            if 'y' not in nc: y_s[...] += y_part(pl.multiple_of((t - TD0) * 2 * CB, 2 * CB), 2 * CB)

    loop(0, TE0 - 1, step)

    y = y_s[...]
    for c0, cw, sl in (last[i] for i in ORD):
        if True:
            wait_on(w2t_v.at[:, :, pl.ds(c0, cw)], sl)
        if True:
            if 'y' not in nc: y = y + y_part(c0, cw)
    y = y[0:B]
    g = y * jax.nn.sigmoid(y)
    out_ref[...] = (x_v[...].astype(F32) + s_s[0:B, :] * g).astype(out_ref.dtype)


@jax.jit
def pallas_recurrent_scan__sliding_block_cached__dense_activation_gelu__decode_kernel(A_x, A_k_cache, A_v_cache, A_wq, A_wo, B_x, B_w1, B_b1, B_w2, B_b2):
    KR = 32
    LOOK = 3
    EX = 0
    TAIL = (256,256)
    NOCOMP = False
    UW = 3
    UK = 1
    NSEM = 5
    SH = 0
    ORD = (0,2,1,3)
    B, Sq, D = A_x.shape
    _, Hkv, Sk, Dh = A_k_cache.shape
    W = min(4096, max(256, Sk // 4))
    HD = A_wq.shape[1]
    F = B_w1.shape[1]
    R = D // NP
    NG = B * Hkv // NP
    any_spec = pl.BlockSpec(memory_space=pl.ANY)
    out = pl.pallas_call(
        functools.partial(_kernel, W=W, KR=KR, LOOK=LOOK, EX=EX, TAIL=TAIL, NOCOMP=NOCOMP, UW=UW, UK=UK, SH=SH, ORD=ORD),
        in_specs=[any_spec] * 9,
        out_specs=pl.BlockSpec(memory_space=pltpu.VMEM),
        out_shape=jax.ShapeDtypeStruct((B, D), A_x.dtype),
        scratch_shapes=[
            pltpu.VMEM((B, D), BF16),
            pltpu.VMEM((F // 128, 128), BF16),
            pltpu.VMEM((D,), BF16),
            pltpu.VMEM((NP, R, HD), BF16),
            pltpu.VMEM((NP, R, F), BF16),
            pltpu.VMEM((NP, R, F), BF16),
            pltpu.VMEM((NP, R, HD), BF16),
            pltpu.VMEM((4, NP, W, Dh), BF16),
            pltpu.VMEM((4, NP, W, Dh), BF16),
            pltpu.VMEM((16, D), BF16),
            pltpu.VMEM((B * HD // Dh, Dh), F32),
            pltpu.VMEM((B * HD // Dh, Dh), F32),
            pltpu.VMEM((F // 128, 128), F32),
            pltpu.VMEM((16, F), BF16),
            pltpu.VMEM((8, D), F32),
            pltpu.VMEM((8, D), F32),
            pltpu.VMEM((8, W), F32),
            pltpu.VMEM((8, Dh), F32),
            pltpu.SemaphoreType.DMA((NSEM,)),
        ],
        compiler_params=pltpu.CompilerParams(vmem_limit_bytes=80 * 2**20, disable_bounds_checks=True),
    )(A_x.reshape(B, D), A_k_cache.reshape(NG, NP, Sk, Dh), A_v_cache.reshape(NG, NP, Sk, Dh),
      A_wq.reshape(NP, R, HD), A_wo.T.reshape(NP, R, HD), B_w1.reshape(NP, R, F),
      B_b1.reshape(F // 128, 128), B_w2.T.reshape(NP, R, F), B_b2)
    return out.reshape(B, Sq, D)
```

```python
import functools

import jax
import jax.numpy as jnp
from jax import lax
import jax.experimental.pallas as pl
import jax.experimental.pallas.tpu as pltpu

F32 = jnp.float32
BF16 = jnp.bfloat16
NT = (((1,), (1,)), ((), ()))

NP = 4
RB = 8
CB = 512
KR = 32
CPG = 8
LOOK = 3
NSLOT = 4


def _loop(lo, hi, fn, unroll=1):
    def body(i, carry):
        fn(i)
        return carry

    lax.fori_loop(lo, hi, body, 0, unroll=unroll)


def _kernel(x_hbm, k_hbm, v_hbm, wq_hbm, wot_hbm, w1_hbm, b1_hbm, w2t_hbm, b2_hbm,
            out_ref,
            x_v, b1_v, b2_v, wq_v, w1_v, w2t_v, wot_v, kbuf, vbuf,
            xn_s, q_s, o_s, b1_s, h_s, y_s, s_s, p_s, l_s, sem, *, W):
    NG, _, Sk, Dh = k_hbm.shape
    _, R, F = w1_hbm.shape
    HD = wq_hbm.shape[2]
    B, D = x_v.shape
    Hq = HD // Dh
    NB = R // RB
    CR = W // CPG
    TPB = CB // Dh
    nq, nf = HD // CB, F // CB
    assert R % (2 * RB) == 0 and CR % KR == 0 and nq % 2 == 0 and nq <= CPG
    assert HD == nq * CB and F == HD + CB and B * Hq == 2 * NP * NG

    T_KV = NB // 2
    T_WO = T_KV + NG * CPG
    T_W2 = T_WO + nq // 2
    T_END = T_W2 + nq // 2 - 1
    last = [(HD - 2 * CB, CB, 0, T_END % NSLOT),
            (HD - CB, CB, 1, (T_END + 1) % NSLOT),
            (HD, CB // 2, 0, (T_END + 2) % NSLOT),
            (HD + CB // 2, CB // 2, 1, NSLOT)]

    def cols(j, width):
        return pl.ds(pl.multiple_of(j * width, width), width)

    def start_w(src, dst, band, columns, queue, slot):
        sl = (slice(None), cols(band, RB), columns)
        pltpu.make_async_copy(src.at[sl], dst.at[sl], sem.at[slot]).start(priority=queue)

    def issue(t):
        slot = t & (NSLOT - 1)

        @pl.when(t < T_KV)
        def _():
            def band(i):
                for j in range(nf):
                    if j < nq:
                        start_w(wq_hbm, wq_v, t * 2 + i, pl.ds(j * CB, CB), 0, slot)
                    start_w(w1_hbm, w1_v, t * 2 + i, pl.ds(j * CB, CB), 1, slot)
            _loop(0, 2, band)

        @pl.when((t >= T_KV) & (t < T_WO))
        def _():
            u = t - T_KV
            g = lax.shift_right_logical(u, 3)
            base = (u & (CPG - 1)) * CR

            def rows(i):
                off = pl.multiple_of(base + i * KR, KR)
                src = pl.ds(Sk - W + off, KR)
                dst = pl.ds(off, KR)
                pltpu.make_async_copy(k_hbm.at[g, :, src], kbuf.at[g & (NSLOT - 1), :, dst],
                                      sem.at[slot]).start(priority=0)
                pltpu.make_async_copy(v_hbm.at[g, :, src], vbuf.at[g & (NSLOT - 1), :, dst],
                                      sem.at[slot]).start(priority=1)
            _loop(0, CR // KR, rows)

        for src, dst, t0, t1 in ((wot_hbm, wot_v, T_WO, T_W2), (w2t_hbm, w2t_v, T_W2, T_END)):
            @pl.when((t >= t0) & (t < t1))
            def _():
                def band(i):
                    for queue in range(2):
                        start_w(src, dst, i, cols((t - t0) * 2 + queue, CB), queue, slot)
                _loop(0, NB, band, 3)

        for n in range(2):
            @pl.when(t == T_END + n)
            def _():
                def band(i):
                    for c0, width, queue, sl in last[2 * n:2 * n + 2]:
                        start_w(w2t_hbm, w2t_v, i, pl.ds(c0, width), queue, sl)
                _loop(0, NB, band, 3)

    def wait_for(dst, slot):
        pltpu.make_async_copy(dst, dst, sem.at[slot]).wait()

    def wait(t):
        slot = t & (NSLOT - 1)

        @pl.when(t < T_KV)
        def _():
            wait_for(wq_v.at[:, cols(t, 2 * RB)], slot)
            wait_for(w1_v.at[:, cols(t, 2 * RB)], slot)

        @pl.when((t >= T_KV) & (t < T_WO))
        def _():
            u = t - T_KV
            g = lax.shift_right_logical(u, 3) & (NSLOT - 1)
            wait_for(kbuf.at[g, :, cols(u & (CPG - 1), CR)], slot)
            wait_for(vbuf.at[g, :, cols(u & (CPG - 1), CR)], slot)

        for dst, t0, t1 in ((wot_v, T_WO, T_W2), (w2t_v, T_W2, T_END)):
            @pl.when((t >= t0) & (t < t1))
            def _():
                wait_for(dst.at[:, :, cols(t - t0, 2 * CB)], slot)

    small = [pltpu.make_async_copy(src, dst, sem.at[LOOK - 1])
             for src, dst in ((x_hbm, x_v), (b1_hbm, b1_v), (b2_hbm, b2_v))]
    _loop(0, LOOK, issue)
    for copy in small:
        copy.start()
    s_s[...] = jnp.zeros(s_s.shape, F32)
    o_s[...] = jnp.zeros(o_s.shape, F32)

    def layernorm():
        for copy in small:
            copy.wait()
        x = x_v[...].astype(F32)
        xc = x - jnp.mean(x, axis=-1, keepdims=True)
        xn = xc / jnp.sqrt(jnp.mean(xc * xc, axis=-1, keepdims=True) + 1e-5)
        xn_s[...] = jnp.concatenate([xn, jnp.zeros((16 - B, D), F32)], axis=0).astype(BF16)
        b1_s[...] = b1_v[...].astype(F32)
        y_s[...] = jnp.broadcast_to(b2_v[...].astype(F32).reshape(1, D), y_s.shape)

    def q_block(j):
        q = jnp.dot(xn_s[...], wq_v[:, :, cols(j, CB)].reshape(D, CB), preferred_element_type=F32)
        for i in range(TPB):
            q_s[pl.ds(j * TPB + i, B, stride=Hq), :] = q[0:B, i * Dh:(i + 1) * Dh]

    def h_block(j):
        h = jnp.dot(xn_s[...], w1_v[:, :, cols(j, CB)].reshape(D, CB), preferred_element_type=F32)
        bias = jnp.concatenate(
            [jnp.broadcast_to(b1_s[pl.ds(j * TPB + i, 1), :], (16, Dh)) for i in range(TPB)], axis=1)
        h_s[:, cols(j, CB)] = jax.nn.gelu(h + bias, approximate=True).astype(BF16)

    def y_part(columns):
        return lax.dot_general(h_s[:, columns], w2t_v[:, :, columns].reshape(D, columns.size), NT,
                               preferred_element_type=F32)[0:8]

    def s_part(j):
        pad = jnp.zeros((8 - B, Dh), F32)
        o = jnp.concatenate(
            [jnp.concatenate([o_s[pl.ds(j * 2 * TPB + i, B, stride=Hq), :], pad], axis=0)
             for i in range(2 * TPB)], axis=1).astype(BF16)
        return lax.dot_general(o, wot_v[:, :, cols(j, 2 * CB)].reshape(D, 2 * CB), NT,
                               preferred_element_type=F32)

    def half_head(u):
        g = lax.shift_right_logical(u, 3)
        j = lax.shift_right_logical(u, 1) & (NP - 1)
        rows = cols(g, 8)

        @pl.when((u & 1) == 0)
        def _():
            s = lax.dot_general(q_s[rows, :].astype(BF16), kbuf[g & (NSLOT - 1), j], NT,
                                preferred_element_type=F32) * (Dh ** -0.5)
            p = jnp.exp(s - jnp.max(s, axis=-1, keepdims=True))
            l_s[...] = jnp.broadcast_to(jnp.sum(p, axis=-1, keepdims=True), l_s.shape)
            p_s[...] = p

        @pl.when((u & 1) == 1)
        def _():
            o = jnp.dot(p_s[...].astype(BF16), vbuf[g & (NSLOT - 1), j],
                        preferred_element_type=F32) / l_s[...]
            row = lax.broadcasted_iota(jnp.int32, (8, Dh), 0)
            o_s[rows, :] = jnp.where(lax.shift_right_logical(row, 1) == j, o, o_s[rows, :])

    def step(t):
        wait(t)
        issue(t + LOOK)
        u = t - T_KV

        @pl.when(t == LOOK - 1)
        def _():
            layernorm()

        @pl.when((u >= 0) & (u < nq))
        def _():
            q_block(u)

        @pl.when((u >= 0) & (u < nf))
        def _():
            h_block(u)

        n = NG * CPG
        lo = jnp.where(u < n, u - CPG, 2 * u - n - CPG + 2)
        hi = jnp.where(u < n - 1, u - CPG + 1, 2 * u - n - CPG + 4)
        _loop(jnp.clip(lo, 0, n), jnp.clip(hi, 0, n), half_head)

        @pl.when((t >= T_WO) & (t < T_W2))
        def _():
            s_s[...] += s_part(t - T_WO)

        @pl.when(t >= T_W2)
        def _():
            y_s[...] += y_part(cols(t - T_W2, 2 * CB))

    _loop(0, T_END, step)

    y = y_s[...]
    for c0, width, _, sl in (last[0], last[2], last[1], last[3]):
        wait_for(w2t_v.at[:, :, pl.ds(c0, width)], sl)
        y = y + y_part(pl.ds(c0, width))
    y = y[0:B]
    out = x_v[...].astype(F32) + s_s[0:B, :] * (y * jax.nn.sigmoid(y))
    out_ref[...] = out.astype(out_ref.dtype)


@jax.jit
def pallas_recurrent_scan__sliding_block_cached__dense_activation_gelu__decode_kernel(
    A_x: jax.Array,
    A_k_cache: jax.Array,
    A_v_cache: jax.Array,
    A_wq: jax.Array,
    A_wo: jax.Array,
    B_x: jax.Array,
    B_w1: jax.Array,
    B_b1: jax.Array,
    B_w2: jax.Array,
    B_b2: jax.Array,
):
    del B_x
    B, Sq, D = A_x.shape
    _, Hkv, Sk, Dh = A_k_cache.shape
    W = min(4096, max(256, Sk // 4))
    HD = A_wq.shape[1]
    F = B_w1.shape[1]
    R = D // NP
    NG = B * Hkv // NP
    out = pl.pallas_call(
        functools.partial(_kernel, W=W),
        in_specs=[pl.BlockSpec(memory_space=pl.ANY)] * 9,
        out_specs=pl.BlockSpec(memory_space=pltpu.VMEM),
        out_shape=jax.ShapeDtypeStruct((B, D), A_x.dtype),
        scratch_shapes=[
            pltpu.VMEM((B, D), BF16),
            pltpu.VMEM((F // 128, 128), BF16),
            pltpu.VMEM((D,), BF16),
            pltpu.VMEM((NP, R, HD), BF16),
            pltpu.VMEM((NP, R, F), BF16),
            pltpu.VMEM((NP, R, F), BF16),
            pltpu.VMEM((NP, R, HD), BF16),
            pltpu.VMEM((NSLOT, NP, W, Dh), BF16),
            pltpu.VMEM((NSLOT, NP, W, Dh), BF16),
            pltpu.VMEM((16, D), BF16),
            pltpu.VMEM((B * HD // Dh, Dh), F32),
            pltpu.VMEM((B * HD // Dh, Dh), F32),
            pltpu.VMEM((F // 128, 128), F32),
            pltpu.VMEM((16, F), BF16),
            pltpu.VMEM((8, D), F32),
            pltpu.VMEM((8, D), F32),
            pltpu.VMEM((8, W), F32),
            pltpu.VMEM((8, Dh), F32),
            pltpu.SemaphoreType.DMA((NSLOT + 1,)),
        ],
        compiler_params=pltpu.CompilerParams(
            vmem_limit_bytes=80 * 2**20, disable_bounds_checks=True),
    )(
        A_x.reshape(B, D),
        A_k_cache.reshape(NG, NP, Sk, Dh),
        A_v_cache.reshape(NG, NP, Sk, Dh),
        A_wq.reshape(NP, R, HD),
        A_wo.T.reshape(NP, R, HD),
        B_w1.reshape(NP, R, F),
        B_b1.reshape(F // 128, 128),
        B_w2.T.reshape(NP, R, F),
        B_b2,
    )
    return out.reshape(B, Sq, D)
```
